```python
import os as _os
_os.environ.setdefault("JAX_PLATFORMS", "cpu")
import jax
import jax.numpy as jnp

def _softmax(x, axis=-1):
    return jax.nn.softmax(x, axis=axis)
def _gelu(x):
    return jax.nn.gelu(x, approximate=True)
def _silu(x):
    return jax.nn.silu(x)
def _sigmoid(x):
    return jax.nn.sigmoid(x)
def _layernorm(x, axis=-1, eps=1e-5):
    m = jnp.mean(x, axis=axis, keepdims=True)
    v = jnp.var(x, axis=axis, keepdims=True)
    return (x - m) / jnp.sqrt(v + eps)
def _scatter_add(tgt, idx, src, axis=0):
    return tgt.at[idx].add(src)
def _segment_sum(src, seg, n):
    return jax.ops.segment_sum(src, seg, n)
class _Rng:
    def __init__(self, key):
        self._k = key
    def _next(self):
        self._k, sub = jax.random.split(self._k)
        return sub
    def normal(self, shape):
        return jax.random.normal(self._next(), shape, dtype=jnp.bfloat16)
    def randint(self, lo, hi, shape):
        return jax.random.randint(self._next(), shape, lo, hi, dtype=jnp.int32)
    def uniform(self, shape, lo=0.0, hi=1.0):
        return jax.random.uniform(self._next(), shape, jnp.bfloat16, lo, hi)
    def permutation(self, n):
        return jax.random.permutation(self._next(), n)


kernel_name = 'recurrent_scan__mha_block__swiglu_ffn__prompt'

def setup_inputs():
    _rng = _Rng(jax.random.key(int.from_bytes(__import__("os").urandom(4), "little")))
    _w = (lambda a: (lambda t: t.astype(jnp.bfloat16) if jnp.issubdtype(t.dtype, jnp.floating) else t)(jnp.asarray(a)))
    def _A_setup():
        B, S, D, H = 1, 2048, 640, 32
        return {
            "x": _w((lambda *s: _rng.normal(s) * 0.05)(B, S, D)),
            "wqkv": _w((lambda *s: _rng.normal(s) * 0.05)(D, 3 * D)),
            "wo": _w((lambda *s: _rng.normal(s) * 0.05)(D, D)),
        }
    _A_in = _A_setup()

    def _B_setup():
        B, S, D, F = 1, 2048, 640, 1728
        return {
            "x": _w((lambda *s: _rng.normal(s) * 0.05)(B, S, D)),
            "w_gate": _w((lambda *s: _rng.normal(s) * 0.05)(D, F)),
            "w_up": _w((lambda *s: _rng.normal(s) * 0.05)(D, F)),
            "w_down": _w((lambda *s: _rng.normal(s) * 0.05)(F, D)),
        }
    _B_in = _B_setup()

    return {
        "A_x": _A_in["x"],
        "A_wqkv": _A_in["wqkv"],
        "A_wo": _A_in["wo"],
        "B_x": _B_in["x"],
        "B_w_gate": _B_in["w_gate"],
        "B_w_up": _B_in["w_up"],
        "B_w_down": _B_in["w_down"],
    }

def reference(A_x, A_wqkv, A_wo, B_x, B_w_gate, B_w_up, B_w_down):
    def _A_ref(x, wqkv, wo):
        B, S, D = x.shape
        H = 32
        Dh = D // H
        qkv = (lambda x, *d: x.transpose(*d))((x @ wqkv).reshape(B, S, 3, H, Dh), 2, 0, 3, 1, 4)
        q, k, v = qkv[0], qkv[1], qkv[2]
        scores = jnp.einsum("bhqd,bhkd->bhqk", q, k) * (Dh ** -0.5)
        p = _softmax(scores, axis=-1)
        o = jnp.einsum("bhqk,bhkd->bhqd", p, v)
        return (lambda x, *d: x.transpose(*d))(o, 0, 2, 1, 3).reshape(B, S, D) @ wo

    def _B_ref(x, w_gate, w_up, w_down):
        g = _silu(x @ w_gate)
        u = x @ w_up
        return (g * u) @ w_down

    x = A_x
    xn = _layernorm(x, axis=-1)
    s = _A_ref(xn, A_wqkv, A_wo)
    g = _silu(_B_ref(xn, B_w_gate, B_w_up, B_w_down))
    return x + s * g
```

```python
import functools
import math

import jax
import jax.numpy as jnp
from jax import lax
import jax.experimental.pallas as pl
import jax.experimental.pallas.tpu as pltpu

S = 2048
D = 640
H = 32
DH = 20
F = 1728
EPS = 1e-5

TQ = 512
TK = 128
NQ = S // TQ
NC = S // TK
RB = 256

NN = (((1,), (0,)), ((), ()))
NT = (((1,), (1,)), ((), ()))
F32 = jnp.float32
BF16 = jnp.bfloat16


def _silu(x):
    return x * (1.0 / (1.0 + jnp.exp(-x)))


def _kernel(x_hbm, wqkv_hbm, wo_hbm, wg_hbm, wu_hbm, wd_hbm, out_hbm,
            x_v, wqkv_v, wo_v, wg_v, wu_v, wd_v,
            xn_v, k_v, q_v, vt_v, ot_v, s0, s1, m0, m1, out_v, sems):
    copies = [
        pltpu.make_async_copy(x_hbm, x_v, sems.at[0]),
        pltpu.make_async_copy(wqkv_hbm, wqkv_v, sems.at[1]),
        pltpu.make_async_copy(wg_hbm, wg_v, sems.at[2]),
        pltpu.make_async_copy(wu_hbm, wu_v, sems.at[3]),
        pltpu.make_async_copy(wd_hbm, wd_v, sems.at[4]),
        pltpu.make_async_copy(wo_hbm, wo_v, sems.at[5]),
    ]
    for c in copies:
        c.start()
    copies[0].wait()

    def ln_body(i, carry):
        r0 = pl.multiple_of(i * RB, RB)
        x = x_v[pl.ds(r0, RB), :].astype(F32)
        mu = jnp.mean(x, axis=-1, keepdims=True)
        xc = x - mu
        var = jnp.mean(xc * xc, axis=-1, keepdims=True)
        xn_v[pl.ds(r0, RB), :] = (xc * lax.rsqrt(var + EPS)).astype(BF16)
        return carry
    lax.fori_loop(0, S // RB, ln_body, 0)

    copies[1].wait()

    qscale = DH ** -0.5 * math.log2(math.e)
    wvt = wqkv_v[:, 2 * D:3 * D].T

    def proj_body(i, carry):
        r0 = pl.multiple_of(i * RB, RB)
        xn = xn_v[pl.ds(r0, RB), :]
        qk = jnp.dot(xn, wqkv_v[:, 0:2 * D], preferred_element_type=F32)
        lane = lax.broadcasted_iota(jnp.int32, (RB, 128), 1)
        lo = lane < 64
        qg = [qk[:, g * 128:(g + 1) * 128] * qscale for g in range(5)]
        kg = [qk[:, D + g * 128:D + (g + 1) * 128] for g in range(5)]
        for g in range(5):
            q_v[g, pl.ds(r0, RB), :] = qg[g].astype(BF16)
            k_v[g, pl.ds(r0, RB), :] = kg[g].astype(BF16)
        for g in range(4):
            q_v[5 + g, pl.ds(r0, RB), :] = jnp.where(lo, qg[g + 1], qg[g]).astype(BF16)
            k_v[5 + g, pl.ds(r0, RB), :] = jnp.where(lo, kg[g + 1], kg[g]).astype(BF16)
        vt = lax.dot_general(wvt, xn, NT, preferred_element_type=F32)
        vt_v[:, :, pl.ds(r0, RB)] = vt.reshape(H // 2, 2 * DH, RB)
        return carry
    lax.fori_loop(0, S // RB, proj_body, 0)

    NIT = H * NQ

    def qk_operands(t):
        e = t % 2
        qi = (t // 2) % NQ
        j = t // (2 * NQ)
        col = (2 * j + e) * DH
        start = col % 128
        g = col // 128
        g = jnp.where(start + DH > 128, g + 5, g)
        q0 = pl.multiple_of(qi * TQ, TQ)
        lane = lax.broadcasted_iota(jnp.int32, (TQ, 128), 1)
        msk = ((lane - start) & 127) < DH
        q = q_v[g, pl.ds(q0, TQ), :]
        q = jnp.where(msk, q, jnp.zeros_like(q))
        return g, q

    def qk_chunk(g, q, c, s_ref, mx):
        s = lax.dot_general(k_v[g, c * TK:(c + 1) * TK, :], q, NT,
                            preferred_element_type=F32)
        s_ref[c * TK:(c + 1) * TK, :] = s
        mc = jnp.max(s.reshape(TK // 8, 8, TQ), axis=0)
        return mc if mx is None else jnp.maximum(mx, mc)

    def finish_max(mx, m_ref):
        m_ref[...] = jnp.broadcast_to(jnp.max(mx, axis=0, keepdims=True), (8, TQ))

    def step(t, e, sa, ma, sb, mb):
        qi = (t // 2) % NQ
        j = t // (2 * NQ)
        q0 = pl.multiple_of(qi * TQ, TQ)
        g, q = qk_operands(jnp.minimum(t + 1, NIT - 1))
        m = ma[0:1, :]
        w0 = 16 * e
        row = lax.broadcasted_iota(jnp.int32, (24, TK), 0)
        vmask = (row < DH) if e == 0 else (row >= 4)
        mx = None
        acc = None
        for c in range(NC):
            mx = qk_chunk(g, q, c, sb, mx)
            p = jnp.exp2(sa[c * TK:(c + 1) * TK, :] - m).astype(BF16)
            vt = jnp.where(vmask, vt_v[j, w0:w0 + 24, c * TK:(c + 1) * TK], 1.0)
            d = lax.dot_general(vt, p, NN, preferred_element_type=F32)
            acc = d if acc is None else acc + d
        finish_max(mx, mb)
        if e == 0:
            l = acc[DH:DH + 1, :]
            o = acc * (1.0 / l)
            ot_v[j, 0:DH, pl.ds(q0, TQ)] = o[0:DH, :]
        else:
            l = acc[0:1, :]
            o = acc * (1.0 / l)
            ot_v[j, DH:2 * DH, pl.ds(q0, TQ)] = o[4:24, :]

    g0, q0v = qk_operands(jnp.int32(0))
    mx = None
    for c in range(NC):
        mx = qk_chunk(g0, q0v, c, s0, mx)
    finish_max(mx, m0)

    U = 4

    def att_body(i, carry):
        for u in range(U // 2):
            t = i * U + 2 * u
            step(t, 0, s0, m0, s1, m1)
            step(t + 1, 1, s1, m1, s0, m0)
        return carry
    lax.fori_loop(0, NIT // U, att_body, 0)

    for c in copies[2:]:
        c.wait()

    def out_copy(i):
        r0 = pl.multiple_of(i * RB, RB)
        return pltpu.make_async_copy(out_v.at[pl.ds(r0, RB), :],
                                     out_hbm.at[pl.ds(r0, RB), :], sems.at[6 + i])

    def tail_body(i, carry):
        r0 = pl.multiple_of(i * RB, RB)
        xn = xn_v[pl.ds(r0, RB), :]
        gate = jnp.dot(xn, wg_v[...], preferred_element_type=F32)
        up = jnp.dot(xn, wu_v[...], preferred_element_type=F32)
        hid = (_silu(gate) * up).astype(BF16)
        y = jnp.dot(hid, wd_v[...], preferred_element_type=F32)
        o = ot_v[:, :, pl.ds(r0, RB)].reshape(D, RB).astype(BF16).T
        s = jnp.dot(o, wo_v[...], preferred_element_type=F32)
        x = x_v[pl.ds(r0, RB), :].astype(F32)
        out_v[pl.ds(r0, RB), :] = (x + s * _silu(y)).astype(BF16)
        out_copy(i).start()
        return carry
    lax.fori_loop(0, S // RB, tail_body, 0)

    for i in range(S // RB):
        out_copy(i).wait()


@jax.jit
def pallas_recurrent_scan__mha_block__swiglu_ffn__prompt_kernel(
    A_x: jax.Array,
    A_wqkv: jax.Array,
    A_wo: jax.Array,
    B_x: jax.Array,
    B_w_gate: jax.Array,
    B_w_up: jax.Array,
    B_w_down: jax.Array,
):
    del B_x
    x = A_x.reshape(S, D)
    any_spec = pl.BlockSpec(memory_space=pl.ANY)
    out = pl.pallas_call(
        _kernel,
        out_shape=jax.ShapeDtypeStruct((S, D), BF16),
        in_specs=[any_spec] * 6,
        out_specs=any_spec,
        scratch_shapes=[
            pltpu.VMEM((S, D), BF16),
            pltpu.VMEM((D, 3 * D), BF16),
            pltpu.VMEM((D, D), BF16),
            pltpu.VMEM((D, F), BF16),
            pltpu.VMEM((D, F), BF16),
            pltpu.VMEM((F, D), BF16),
            pltpu.VMEM((S, D), BF16),
            pltpu.VMEM((9, S, 128), BF16),
            pltpu.VMEM((9, S, 128), BF16),
            pltpu.VMEM((H // 2, 2 * DH, S), F32),
            pltpu.VMEM((H // 2, 2 * DH, S), F32),
            pltpu.VMEM((S, TQ), F32),
            pltpu.VMEM((S, TQ), F32),
            pltpu.VMEM((8, TQ), F32),
            pltpu.VMEM((8, TQ), F32),
            pltpu.VMEM((S, D), BF16),
            pltpu.SemaphoreType.DMA((6 + S // RB,)),
        ],
        compiler_params=pltpu.CompilerParams(vmem_limit_bytes=100 * 1024 * 1024),
    )(x, A_wqkv, A_wo, B_w_gate, B_w_up, B_w_down)
    return out.reshape(1, S, D)
```

```python
import math

import jax
import jax.numpy as jnp
from jax import lax
import jax.experimental.pallas as pl
import jax.experimental.pallas.tpu as pltpu

S = 2048
D = 640
H = 32
DH = 20
F = 1728
FM = 1664
EPS = 1e-5
LOG2E = math.log2(math.e)

NN = (((1,), (0,)), ((), ()))
NT = (((1,), (1,)), ((), ()))
F32 = jnp.float32
BF16 = jnp.bfloat16
U32 = jnp.uint32
I32 = jnp.int32
I8 = jnp.int8

NP = H // 2
FB = S // NP
NQT = S // 128
NV = 2 * NQT
NR = 8
QL = 1024
PL = 128
UQ = S // QL
PP = S // PL
LU = 3 * UQ
QE = 1.04
FH = 2
NFT = 205
CBR = 16
CGAP = 4.0
LFE = 0.6
TLAG = 1.5
TB = 256
NO = S // TB
OUTS = [(0, 768, 0, D), (768, 1536, 0, D), (1536, 1792, 0, D), (1792, S, 0, 384), (1792, S, 384, D)]

RB = 256
QB = 128
MH = 16
XCH = [0, 1, 2, 4, 8]
B1, B2, B3, B4, NV0, B5 = 3, 8, 15, 26, 30, 14
LNS = 7
VKEEP = 3
NX = len(XCH) - 1
SEM_W = NX
SEM_O = NX + 8

BASE = 242.0
YMAX = 2770.0
MAGIC = 12582912.0


def _silu(x):
    return x * pl.reciprocal(1.0 + jnp.exp2(x * (-LOG2E)), approx=True)


def _pack(x):
    return pltpu.bitcast(x.astype(BF16), U32)


def _unpack(x):
    return pltpu.bitcast(x, BF16)


def _colmax8(s):
    return jnp.max(s.reshape(s.shape[0] // 8, 8, s.shape[1]), axis=0)


def _digits(v, e, is_q):
    n = v.shape[1]
    row = lax.broadcasted_iota(I32, (8, n), 0)
    if e == 0:
        v = jnp.concatenate([v[0:16], jnp.where(row < 4, v[16:24], 0.0)], axis=0)
    else:
        v = jnp.concatenate([jnp.where(row >= 4, v[0:8], 0.0), v[8:24]], axis=0)
    amax = jnp.maximum(jnp.max(jnp.abs(v), axis=0, keepdims=True), 1e-30)
    z = v * ((YMAX / BASE) * pl.reciprocal(amax, approx=True))
    hi = z + MAGIC
    a = hi - MAGIC
    f = z - a
    top = a * 11.0 + MAGIC
    lo = f * BASE + MAGIC
    lh = f * BASE ** 0.5 + MAGIC
    mid = [hi, lo] if is_q else [lo, hi]
    w = jnp.concatenate([top, top] + mid + [lh, jnp.zeros((8, n), F32)], axis=0)
    return amax, pltpu.bitcast(w, I32)


def _kernel(x_hbm, wqkv_hbm, wo_hbm, wg_hbm, wu_hbm, wd_hbm, out_hbm,
            x_v, wqkv_v, wo_v, wgu_v, wd_v,
            xn_p, wgu_p, wd_p, wt_p, sc_v, k_p, ck_v, cb0, cb1, q_p, cq_v, ve_v, ot_v,
            sr_v, mr_v, h_p, g_v, out_v, sems):
    def x_copy(i):
        r0, r1 = XCH[i] * RB, XCH[i + 1] * RB
        return pltpu.make_async_copy(x_hbm.at[r0:r1, :], x_v.at[r0:r1, :], sems.at[i])

    def out_copy(i):
        r0, r1, c0, c1 = OUTS[i]
        return pltpu.make_async_copy(out_v.at[r0:r1, c0:c1], out_hbm.at[r0:r1, c0:c1], sems.at[SEM_O + i])

    w_copies = [
        pltpu.make_async_copy(wqkv_hbm.at[:, 2 * D:3 * D], wqkv_v.at[:, 2 * D:3 * D], sems.at[SEM_W]),
        pltpu.make_async_copy(wqkv_hbm.at[:, D:2 * D], wqkv_v.at[:, D:2 * D], sems.at[SEM_W + 1]),
        pltpu.make_async_copy(wqkv_hbm.at[:, 0:D], wqkv_v.at[:, 0:D], sems.at[SEM_W + 2]),
        pltpu.make_async_copy(wg_hbm, wgu_v.at[0:F, :], sems.at[SEM_W + 3]),
        pltpu.make_async_copy(wu_hbm.at[FM:F, :], wgu_v.at[F:F + 64, :], sems.at[SEM_W + 4]),
        pltpu.make_async_copy(wu_hbm.at[0:FM, :], wgu_v.at[F + 64:2 * F, :], sems.at[SEM_W + 5]),
        pltpu.make_async_copy(wd_hbm, wd_v, sems.at[SEM_W + 6]),
        pltpu.make_async_copy(wo_hbm, wo_v, sems.at[SEM_W + 7]),
    ]

    def layernorm(i):
        r0 = i * RB
        x = x_v[r0:r0 + RB, :].astype(F32)
        mu = jnp.sum(x, axis=-1, keepdims=True) * (1.0 / D)
        xc = x - mu
        var = jnp.sum(xc * xc, axis=-1, keepdims=True) * (1.0 / D)
        xn_p[r0 // 2:(r0 + RB) // 2, :] = _pack(xc * lax.rsqrt(var + EPS))

    def qk_piece(is_q, i, n):
        r0 = i * QB
        xn = _unpack(xn_p[r0 // 2:(r0 + QB) // 2, :])
        w0 = ((0 if is_q else D) + n * MH * DH) // 2
        yt = lax.dot_general(_unpack(wt_p[w0:w0 + MH * DH // 2, :]), xn, NT, preferred_element_type=F32)
        for hl in range(MH):
            h = n * MH + hl
            g0 = (hl * DH) // 8
            amax, w = _digits(yt[8 * g0:8 * g0 + 24], h % 2, is_q)
            if is_q:
                q_p[h, :, r0:r0 + QB] = pltpu.bitcast(w.astype(I8), U32)
                cq_v[h // 2, h % 2:h % 2 + 1, r0:r0 + QB] = amax * (BASE / YMAX ** 2 * DH ** -0.5 * LOG2E)
            else:
                k_p[h, r0 // 4:(r0 + QB) // 4, :] = pltpu.bitcast(w.astype(jnp.int16).T.astype(I8), U32)
                sc_v[h:h + 1, r0:r0 + QB] = amax
        if not is_q and (n + 1) * MH == H:
            ck_v[r0:r0 + QB, :] = sc_v[:, r0:r0 + QB].T

    def store_v(r0, n, y):
        yt = y.T
        row = lax.broadcasted_iota(I32, (8, RB), 0)
        for r in range(16):
            j, g = (16 * n + r) // 5, (16 * n + r) % 5
            v = yt[8 * r:8 * r + 8]
            if g < 2:
                ve_v[2 * j, 8 * g:8 * g + 8, r0:r0 + RB] = v
            elif g > 2:
                ve_v[2 * j + 1, 8 * g - 16:8 * g - 8, r0:r0 + RB] = v
            else:
                ve_v[2 * j, 16:24, r0:r0 + RB] = jnp.where(row < 4, v, 1.0)
                ve_v[2 * j + 1, 0:8, r0:r0 + RB] = jnp.where(row >= 4, v, 1.0)

    pend = []

    def v_piece(i, n):
        xn = _unpack(xn_p[i * RB // 2:(i + 1) * RB // 2, :])
        y = jnp.dot(xn, wqkv_v[:, 2 * D + n * 128:2 * D + (n + 1) * 128], preferred_element_type=F32)
        pend.append((i * RB, n, y))
        if len(pend) > 1:
            store_v(*pend.pop(0))

    x_copy(0).start()
    w_copies[0].start()
    x_copy(1).start()
    sc_v[H:128, :] = jnp.zeros((128 - H, S), F32)
    x_copy(0).wait()
    layernorm(0)
    w_copies[0].wait()
    x_copy(2).start()
    x_copy(3).start()
    for c in w_copies[1:]:
        c.start()

    vs = [(i, n) for i in range(S // RB) for n in range(5)]
    for cnt in range(NV0):
        if cnt == B1:
            x_copy(1).wait()
            layernorm(1)
        if cnt == B2:
            x_copy(2).wait()
            layernorm(2)
            layernorm(3)
        if cnt == B3:
            x_copy(3).wait()
            for i in range(4, LNS):
                layernorm(i)
        if cnt == B4:
            w_copies[1].wait()
            w_copies[2].wait()
            for i in range(LNS, S // RB):
                layernorm(i)
            for t in (5, 6, 7, 0, 1, 2, 8, 9, 3, 4):
                wt_p[t * 64:(t + 1) * 64, :] = pltpu.bitcast(wqkv_v[:, t * 128:(t + 1) * 128].T, U32)
        v_piece(*vs.pop(0))
    pieces = [(i, n) for i in range(S // QB) for n in range(H // MH)]
    npc, nv = len(pieces), len(vs)
    wjobs = [(0, t) for t in range(27)] + [(1, t) for t in range(14)]
    for cnt, (i, n) in enumerate(pieces):
        if cnt == B5:
            for c in w_copies[3:]:
                c.wait()
        qk_piece(True, i, n)
        qk_piece(False, i, n)
        while cnt >= B5 and len(wjobs) > 41 * (1.0 - (cnt + 1 - B5) / (npc - B5)):
            kind, t = wjobs.pop(0)
            if kind == 0:
                wgu_p[:, t * 128:(t + 1) * 128] = pltpu.bitcast(wgu_v[t * 128:(t + 1) * 128, :].T, U32)
            else:
                r1 = min(F, (t + 1) * 128)
                wd_p[t * 64:r1 // 2, :] = pltpu.bitcast(wd_v[t * 128:r1, :], U32)
        while nv - len(vs) < (nv - VKEEP) * (cnt + 1) / npc:
            v_piece(*vs.pop(0))
    assert not wjobs
    for v in vs:
        v_piece(*v)
    for p in pend:
        store_v(*p)

    cbuf = (cb0, cb1)

    class CB:
        NPC = S // CBR

        def __init__(self, j, e):
            self.j, self.e, self.n = j, e, 0

        def run_to(self, n_end):
            while self.n < min(n_end, self.NPC):
                r0, r1 = self.n * CBR, (self.n + 1) * CBR
                cbuf[self.e][r0:r1, :] = jnp.take_along_axis(
                    ck_v[r0:r1, :], jnp.full((CBR, 128), 2 * self.j + self.e, I32), axis=1)
                self.n += 1

    class QK:
        def __init__(self, j, n):
            self.j, self.n = j, n

        def run_to(self, n_end):
            while self.n < n_end:
                v, kq = self.n // UQ, self.n % UQ
                j, e, t = self.j + v // NV, (v % NV) // NQT, v % NQT
                r0, r1 = kq * QL, (kq + 1) * QL
                q = pltpu.bitcast(q_p[2 * j + e, :, t * 128:(t + 1) * 128], I8)
                k = pltpu.bitcast(k_p[2 * j + e, r0 // 4:r1 // 4, :], I8)
                s = lax.dot_general(k, q, NN, preferred_element_type=I32).astype(F32)
                s = s * cbuf[e][r0:r1, :]
                sr_v[v % NR, r0:r1, :] = s
                mc = _colmax8(s)
                self.mx = mc if kq == 0 else jnp.maximum(self.mx, mc)
                if r1 == S:
                    mr_v[v % NR] = jnp.broadcast_to(jnp.max(self.mx, axis=0, keepdims=True), (8, 128))
                self.n += 1

    class FFN:
        def __init__(self, j):
            self.n = 0
            self.r0 = j * FB if isinstance(j, int) else pl.multiple_of(j * FB, FB)
            self.p0 = j * (FB // 2) if isinstance(j, int) else pl.multiple_of(j * (FB // 2), FB // 2)
            cols = [("m", 13)]
            for p in range(13):
                cols += [("g", p), ("u", p)]
            self.tiles = [(kind, p, kt) for (kind, p) in cols for kt in range(5)]
            self.tiles += [("d", n, kt) for n in range(5) for kt in range(14)]

        def run_to(self, n_end):
            while self.n < min(n_end, NFT):
                kind, p, kt = self.tiles[self.n]
                self.n += 1
                if kind != "d":
                    xn = _unpack(xn_p[pl.ds(self.p0, FB // 2), kt * 128:(kt + 1) * 128])
                    t = p if kind != "u" else 14 + p
                    w = _unpack(wgu_p[kt * 64:(kt + 1) * 64, t * 128:(t + 1) * 128])
                    d = jnp.dot(xn, w, preferred_element_type=F32)
                    self.y = y = d if kt == 0 else self.y + d
                    if kt == 4:
                        if kind == "g":
                            self.gate = _silu(y)
                        elif kind == "u":
                            h_p[p] = _pack(self.gate * y)
                        else:
                            h_p[13] = _pack(_silu(y) * pltpu.roll(y, 64, 1))
                else:
                    if kt < 13:
                        d = jnp.dot(_unpack(h_p[kt]), _unpack(wd_p[kt * 64:(kt + 1) * 64, p * 128:(p + 1) * 128]),
                                    preferred_element_type=F32)
                    else:
                        d = jnp.dot(_unpack(h_p[13])[:, 0:64], _unpack(wd_p[FM // 2:F // 2, p * 128:(p + 1) * 128]),
                                    preferred_element_type=F32)
                    self.y = d if kt == 0 else self.y + d
                    if kt == 13:
                        g_v[pl.ds(self.r0, FB), p * 128:(p + 1) * 128] = _silu(self.y)

    class Tail:
        def __init__(self):
            self.n = 0

        def run_to(self, n_end):
            while self.n < min(n_end, 25 * NO):
                i, n, kt = self.n // 25, (self.n % 25) // 5, self.n % 5
                r0, r1, c0, c1 = i * TB, (i + 1) * TB, n * 128, (n + 1) * 128
                if self.n % 25 == 0:
                    self.o = ot_v[:, :, r0:r1].reshape(D, TB).astype(BF16).T
                d = jnp.dot(self.o[:, kt * 128:(kt + 1) * 128], wo_v[kt * 128:(kt + 1) * 128, c0:c1],
                            preferred_element_type=F32)
                self.s = d if kt == 0 else self.s + d
                if kt == 4:
                    out_v[r0:r1, c0:c1] = (x_v[r0:r1, c0:c1].astype(F32)
                                           + self.s * g_v[r0:r1, c0:c1]).astype(BF16)
                    for ci, o in enumerate(OUTS):
                        if o[1] == r1 and o[3] == c1:
                            out_copy(ci).start()
                self.n += 1

    def step(j, v, hook):
        e, t = v // NQT, v % NQT
        m8 = mr_v[v % NR]
        cq = jnp.broadcast_to(cq_v[j, e:e + 1, t * 128:(t + 1) * 128], (8, 128))
        acc = None
        for c in range(PP):
            r0, r1 = c * PL, (c + 1) * PL
            hook(v * PP + c)
            s = sr_v[v % NR, r0:r1, :].reshape(PL // 8, 8, 128)
            p = jnp.exp2((s - m8[None]) * cq[None]).reshape(PL, 128)
            d = lax.dot_general(ve_v[2 * j + e, :, r0:r1], p, NN, preferred_element_type=F32)
            acc = d if acc is None else acc + d
        if e == 0:
            o = acc * pl.reciprocal(acc[DH:DH + 1, :], approx=True)
            ot_v[j, 0:DH, t * 128:(t + 1) * 128] = o[0:DH, :]
        else:
            o = acc * pl.reciprocal(acc[0:1, :], approx=True)
            ot_v[j, DH:2 * DH, t * 128:(t + 1) * 128] = o[4:24, :]

    def body(j, last):
        qk, ffn, tail = QK(j, LU), FFN(j), Tail()
        cb1s, cb0s = CB(j, 1), CB(j + 1, 0)
        npos = NV * PP
        lead = LU / UQ + (QE - 1) * NV + 1
        a1 = (NQT - lead - CGAP) * PP
        b0, b1 = (NQT - LU / UQ + 0.5) * PP, (NV - lead - CGAP) * PP

        def hook(n):
            end = LU + min(NV * UQ, int(math.ceil((n + 1) * UQ / PP * QE - 1e-9)))
            if last:
                end = min(end, NV * UQ)
            assert (end - 1) // UQ - NR < n // PP
            assert (end - 1) // UQ < NQT or cb1s.n == CB.NPC
            assert (end - 1) // UQ < NV or cb0s.n == CB.NPC
            qk.run_to(end)
            ffn.run_to(FH + (NFT - FH) * (n + 1) / (npos * (LFE if last else 1.0)))
            cb1s.run_to(int(CB.NPC * (n + 1) / a1))
            if not last:
                if qk.n >= NQT * UQ:
                    cb0s.run_to(int(CB.NPC * (n + 1 - b0) / (b1 - b0)))
            else:
                ready = (max(0, n // PP - NQT) * 128 // TB) * 25
                want = (n / PP - NQT - TB // 128 - TLAG + 1) * 128 / TB * 25
                tail.run_to(min(ready, int(want)))

        for v in range(NV):
            step(j, v, hook)
        assert ffn.n == NFT and (last or qk.n == LU + NV * UQ)
        if last:
            tail.run_to(25 * NO)

    def att_body(j, carry):
        body(j, False)
        return carry

    CB(0, 0).run_to(CB.NPC)
    QK(0, 0).run_to(LU)
    lax.fori_loop(0, NP - 1, att_body, 0)
    body(NP - 1, True)

    for i in range(len(OUTS)):
        out_copy(i).wait()


@jax.jit
def pallas_recurrent_scan__mha_block__swiglu_ffn__prompt_kernel(
    A_x: jax.Array,
    A_wqkv: jax.Array,
    A_wo: jax.Array,
    B_x: jax.Array,
    B_w_gate: jax.Array,
    B_w_up: jax.Array,
    B_w_down: jax.Array,
):
    del B_x
    hbm_spec = pl.BlockSpec(memory_space=pltpu.MemorySpace.HBM)
    out = pl.pallas_call(
        _kernel,
        out_shape=jax.ShapeDtypeStruct((S, D), BF16),
        in_specs=[hbm_spec] * 6,
        out_specs=hbm_spec,
        scratch_shapes=[
            pltpu.VMEM((S, D), BF16),
            pltpu.VMEM((D, 3 * D), BF16),
            pltpu.VMEM((D, D), BF16),
            pltpu.VMEM((2 * F, D), BF16),
            pltpu.VMEM((F, D), BF16),
            pltpu.VMEM((S // 2, D), U32),
            pltpu.VMEM((D // 2, 2 * F), U32),
            pltpu.VMEM((F // 2, D), U32),
            pltpu.VMEM((D, D), U32),
            pltpu.VMEM((128, S), F32),
            pltpu.VMEM((H, S // 4, 128), U32),
            pltpu.VMEM((S, 128), F32),
            pltpu.VMEM((S, 128), F32),
            pltpu.VMEM((S, 128), F32),
            pltpu.VMEM((H, 32, S), U32),
            pltpu.VMEM((NP, 8, S), F32),
            pltpu.VMEM((H, 24, S), F32),
            pltpu.VMEM((NP, 2 * DH, S), F32),
            pltpu.VMEM((NR, S, 128), F32),
            pltpu.VMEM((NR, 8, 128), F32),
            pltpu.VMEM((14, FB // 2, 128), U32),
            pltpu.VMEM((S, D), F32),
            pltpu.VMEM((S, D), BF16),
            pltpu.SemaphoreType.DMA((SEM_O + len(OUTS),)),
        ],
        compiler_params=pltpu.CompilerParams(vmem_limit_bytes=100 * 1024 * 1024),
    )(A_x.reshape(S, D), A_wqkv, A_wo, B_w_gate.T, B_w_up.T, B_w_down)
    return out.reshape(1, S, D)
```

```python
import math

import jax
import jax.numpy as jnp
from jax import lax
import jax.experimental.pallas as pl
import jax.experimental.pallas.tpu as pltpu

S = 2048
D = 640
H = 32
DH = 20
F = 1728
FM = 1664
EPS = 1e-5
LOG2E = math.log2(math.e)

NN = (((1,), (0,)), ((), ()))
NT = (((1,), (1,)), ((), ()))
F32 = jnp.float32
BF16 = jnp.bfloat16
U32 = jnp.uint32
I32 = jnp.int32
I8 = jnp.int8

NP = H // 2
FB = S // NP
NQT = S // 128
NV = 2 * NQT
NR = 8
QL = 1024
PL = 128
UQ = S // QL
PP = S // PL
LU = 3 * UQ
QE = 1.04
FH = 2
NFT = 205
CBR = 16
CGAP = 4.0
LFE = 0.6
TLAG = 1.5
TB = 256
NO = S // TB
OUTS = [(0, 768, 0, D), (768, 1536, 0, D), (1536, 1792, 0, D), (1792, S, 0, 384), (1792, S, 384, D)]

RB = 256
QB = 128
MH = 16
XCH = [0, 1, 2, 4, 8]
B1, B2, B3, B4, NV0, B5 = 3, 8, 16, 26, 30, 14
LNS = 7
VKEEP = 5
VB5 = 2
NX = len(XCH) - 1
SEM_W = NX
SEM_O = NX + 8

BASE = 242.0
YMAX = 2770.0
MAGIC = 12582912.0


def _silu(x):
    return x * pl.reciprocal(1.0 + jnp.exp2(x * (-LOG2E)), approx=True)


def _pack(x):
    return pltpu.bitcast(x.astype(BF16), U32)


def _unpack(x):
    return pltpu.bitcast(x, BF16)


def _colmax8(s):
    return jnp.max(s.reshape(s.shape[0] // 8, 8, s.shape[1]), axis=0)


def _sumsq(w):
    w = w.astype(F32)
    return jnp.broadcast_to(jnp.sum(w * w, axis=0, keepdims=True), (8, w.shape[1]))


def _digits(v, e, is_q):
    n = v.shape[1]
    row = lax.broadcasted_iota(I32, (8, n), 0)
    if e == 0:
        v = jnp.concatenate([v[0:16], jnp.where(row < 4, v[16:24], 0.0)], axis=0)
    else:
        v = jnp.concatenate([jnp.where(row >= 4, v[0:8], 0.0), v[8:24]], axis=0)
    amax = jnp.maximum(jnp.max(jnp.abs(v), axis=0, keepdims=True), 1e-30)
    z = v * ((YMAX / BASE) * pl.reciprocal(amax, approx=True))
    hi = z + MAGIC
    a = hi - MAGIC
    f = z - a
    top = a * 11.0 + MAGIC
    lo = f * BASE + MAGIC
    lh = f * BASE ** 0.5 + MAGIC
    mid = [hi, lo] if is_q else [lo, hi]
    w = jnp.concatenate([top, top] + mid + [lh, jnp.zeros((8, n), F32)], axis=0)
    return amax, pltpu.bitcast(w, I32)


def _kernel(x_hbm, wqkv_hbm, wo_hbm, wg_hbm, wu_hbm, wd_hbm, out_hbm,
            x_v, wqkv_v, wo_v, wgu_v, wd_v,
            xn_p, wgu_p, wd_p, wt_p, sc_v, k_p, ck_v, cb0, cb1, q_p, cq_v, ve_v, ot_v,
            sr_v, mr_v, h_p, g_v, out_v, sems):
    def x_copy(i):
        r0, r1 = XCH[i] * RB, XCH[i + 1] * RB
        return pltpu.make_async_copy(x_hbm.at[r0:r1, :], x_v.at[r0:r1, :], sems.at[i])

    def out_copy(i):
        r0, r1, c0, c1 = OUTS[i]
        return pltpu.make_async_copy(out_v.at[r0:r1, c0:c1], out_hbm.at[r0:r1, c0:c1], sems.at[SEM_O + i])

    w_copies = [
        pltpu.make_async_copy(wqkv_hbm.at[:, 2 * D:3 * D], wqkv_v.at[:, 2 * D:3 * D], sems.at[SEM_W]),
        pltpu.make_async_copy(wqkv_hbm.at[:, D:2 * D], wqkv_v.at[:, D:2 * D], sems.at[SEM_W + 1]),
        pltpu.make_async_copy(wqkv_hbm.at[:, 0:D], wqkv_v.at[:, 0:D], sems.at[SEM_W + 2]),
        pltpu.make_async_copy(wg_hbm, wgu_v.at[0:F, :], sems.at[SEM_W + 3]),
        pltpu.make_async_copy(wu_hbm.at[FM:F, :], wgu_v.at[F:F + 64, :], sems.at[SEM_W + 4]),
        pltpu.make_async_copy(wu_hbm.at[0:FM, :], wgu_v.at[F + 64:2 * F, :], sems.at[SEM_W + 5]),
        pltpu.make_async_copy(wd_hbm, wd_v, sems.at[SEM_W + 6]),
        pltpu.make_async_copy(wo_hbm, wo_v, sems.at[SEM_W + 7]),
    ]

    def layernorm(i):
        r0 = i * RB
        x = x_v[r0:r0 + RB, :].astype(F32)
        mu = jnp.sum(x, axis=-1, keepdims=True) * (1.0 / D)
        xc = x - mu
        var = jnp.sum(xc * xc, axis=-1, keepdims=True) * (1.0 / D)
        xn_p[r0 // 2:(r0 + RB) // 2, :] = _pack(xc * lax.rsqrt(var + EPS))

    def balanced_transpose(t):
        wq = wqkv_v[:, t * 128:(t + 1) * 128]
        wk = wqkv_v[:, D + t * 128:D + (t + 1) * 128]
        nq = pltpu.bitcast(_sumsq(wq), I32)
        nk = pltpu.bitcast(_sumsq(wk), I32)
        ex = (nk - nq + (1 << 24)) >> 25
        ex = jnp.concatenate([ex] * 16, axis=0).T
        bq = pltpu.bitcast((127 + ex) << 23, F32)
        bk = pltpu.bitcast((127 - ex) << 23, F32)
        wt_p[t * 64:(t + 1) * 64, :] = _pack(wq.T.astype(F32) * jnp.concatenate([bq] * 5, axis=1))
        wt_p[(5 + t) * 64:(6 + t) * 64, :] = _pack(wk.T.astype(F32) * jnp.concatenate([bk] * 5, axis=1))

    def qk_piece(is_q, i, n):
        r0 = i * QB
        xn = _unpack(xn_p[r0 // 2:(r0 + QB) // 2, :])
        w0 = ((0 if is_q else D) + n * MH * DH) // 2
        yt = lax.dot_general(_unpack(wt_p[w0:w0 + MH * DH // 2, :]), xn, NT, preferred_element_type=F32)
        for hl in range(MH):
            h = n * MH + hl
            g0 = (hl * DH) // 8
            amax, w = _digits(yt[8 * g0:8 * g0 + 24], h % 2, is_q)
            if is_q:
                q_p[h, :, r0:r0 + QB] = pltpu.bitcast(w.astype(I8), U32)
                cq_v[h // 2, h % 2:h % 2 + 1, r0:r0 + QB] = amax * (BASE / YMAX ** 2 * DH ** -0.5 * LOG2E)
            else:
                k_p[h, r0 // 4:(r0 + QB) // 4, :] = pltpu.bitcast(w.astype(jnp.int16).T.astype(I8), U32)
                sc_v[h:h + 1, r0:r0 + QB] = amax
        if not is_q and (n + 1) * MH == H:
            ck_v[r0:r0 + QB, :] = sc_v[:, r0:r0 + QB].T

    def store_v(r0, n, y):
        yt = y.T
        row = lax.broadcasted_iota(I32, (8, RB), 0)
        for r in range(16):
            j, g = (16 * n + r) // 5, (16 * n + r) % 5
            v = yt[8 * r:8 * r + 8]
            if g < 2:
                ve_v[2 * j, 8 * g:8 * g + 8, r0:r0 + RB] = v
            elif g > 2:
                ve_v[2 * j + 1, 8 * g - 16:8 * g - 8, r0:r0 + RB] = v
            else:
                ve_v[2 * j, 16:24, r0:r0 + RB] = jnp.where(row < 4, v, 1.0)
                ve_v[2 * j + 1, 0:8, r0:r0 + RB] = jnp.where(row >= 4, v, 1.0)

    pend = []

    def v_piece(i, n):
        xn = _unpack(xn_p[i * RB // 2:(i + 1) * RB // 2, :])
        y = jnp.dot(xn, wqkv_v[:, 2 * D + n * 128:2 * D + (n + 1) * 128], preferred_element_type=F32)
        pend.append((i * RB, n, y))
        if len(pend) > 1:
            store_v(*pend.pop(0))

    x_copy(0).start()
    w_copies[0].start()
    x_copy(1).start()
    sc_v[H:128, :] = jnp.zeros((128 - H, S), F32)
    x_copy(0).wait()
    layernorm(0)
    w_copies[0].wait()
    x_copy(2).start()
    x_copy(3).start()
    for c in w_copies[1:]:
        c.start()

    vs = [(i, n) for i in range(S // RB) for n in range(5)]
    for cnt in range(NV0):
        if cnt == B1:
            x_copy(1).wait()
            layernorm(1)
        if cnt == B2:
            x_copy(2).wait()
            layernorm(2)
            layernorm(3)
        if cnt == B3:
            x_copy(3).wait()
            for i in range(4, LNS):
                layernorm(i)
        if cnt == B4:
            w_copies[1].wait()
            w_copies[2].wait()
            for i in range(LNS, S // RB):
                layernorm(i)
            for t in range(5):
                balanced_transpose(t)
        v_piece(*vs.pop(0))
    pieces = [(i, n) for i in range(S // QB) for n in range(H // MH)]
    npc, nv = len(pieces), len(vs)
    wjobs = [(0, t) for t in range(27)] + [(1, t) for t in range(14)]
    for cnt, (i, n) in enumerate(pieces):
        if cnt == B5:
            for _ in range(VB5):
                v_piece(*vs.pop(0))
            for c in w_copies[3:]:
                c.wait()
        qk_piece(True, i, n)
        qk_piece(False, i, n)
        while cnt >= B5 and len(wjobs) > 41 * (1.0 - (cnt + 1 - B5) / (npc - B5)):
            kind, t = wjobs.pop(0)
            if kind == 0:
                wgu_p[:, t * 128:(t + 1) * 128] = pltpu.bitcast(wgu_v[t * 128:(t + 1) * 128, :].T, U32)
            else:
                r1 = min(F, (t + 1) * 128)
                wd_p[t * 64:r1 // 2, :] = pltpu.bitcast(wd_v[t * 128:r1, :], U32)
        while nv - len(vs) - (VB5 if cnt >= B5 else 0) < (nv - VKEEP - VB5) * (cnt + 1) / npc:
            v_piece(*vs.pop(0))
    assert not wjobs
    for v in vs:
        v_piece(*v)
    for p in pend:
        store_v(*p)

    cbuf = (cb0, cb1)

    class CB:
        NPC = S // CBR

        def __init__(self, j, e):
            self.j, self.e, self.n = j, e, 0

        def run_to(self, n_end):
            while self.n < min(n_end, self.NPC):
                r0, r1 = self.n * CBR, (self.n + 1) * CBR
                cbuf[self.e][r0:r1, :] = jnp.take_along_axis(
                    ck_v[r0:r1, :], jnp.full((CBR, 128), 2 * self.j + self.e, I32), axis=1)
                self.n += 1

    class QK:
        def __init__(self, j, n):
            self.j, self.n = j, n

        def run_to(self, n_end):
            while self.n < n_end:
                v, kq = self.n // UQ, self.n % UQ
                j, e, t = self.j + v // NV, (v % NV) // NQT, v % NQT
                r0, r1 = kq * QL, (kq + 1) * QL
                q = pltpu.bitcast(q_p[2 * j + e, :, t * 128:(t + 1) * 128], I8)
                k = pltpu.bitcast(k_p[2 * j + e, r0 // 4:r1 // 4, :], I8)
                s = lax.dot_general(k, q, NN, preferred_element_type=I32).astype(F32)
                s = s * cbuf[e][r0:r1, :]
                sr_v[v % NR, r0:r1, :] = s
                mc = _colmax8(s)
                self.mx = mc if kq == 0 else jnp.maximum(self.mx, mc)
                if r1 == S:
                    mr_v[v % NR] = jnp.broadcast_to(jnp.max(self.mx, axis=0, keepdims=True), (8, 128))
                self.n += 1

    class FFN:
        def __init__(self, j):
            self.n = 0
            self.r0 = j * FB if isinstance(j, int) else pl.multiple_of(j * FB, FB)
            self.p0 = j * (FB // 2) if isinstance(j, int) else pl.multiple_of(j * (FB // 2), FB // 2)
            cols = [("m", 13)]
            for p in range(13):
                cols += [("g", p), ("u", p)]
            self.tiles = [(kind, p, kt) for (kind, p) in cols for kt in range(5)]
            self.tiles += [("d", n, kt) for n in range(5) for kt in range(14)]

        def run_to(self, n_end):
            while self.n < min(n_end, NFT):
                kind, p, kt = self.tiles[self.n]
                self.n += 1
                if kind != "d":
                    xn = _unpack(xn_p[pl.ds(self.p0, FB // 2), kt * 128:(kt + 1) * 128])
                    t = p if kind != "u" else 14 + p
                    w = _unpack(wgu_p[kt * 64:(kt + 1) * 64, t * 128:(t + 1) * 128])
                    d = jnp.dot(xn, w, preferred_element_type=F32)
                    self.y = y = d if kt == 0 else self.y + d
                    if kt == 4:
                        if kind == "g":
                            self.gate = _silu(y)
                        elif kind == "u":
                            h_p[p] = _pack(self.gate * y)
                        else:
                            h_p[13] = _pack(_silu(y) * pltpu.roll(y, 64, 1))
                else:
                    if kt < 13:
                        d = jnp.dot(_unpack(h_p[kt]), _unpack(wd_p[kt * 64:(kt + 1) * 64, p * 128:(p + 1) * 128]),
                                    preferred_element_type=F32)
                    else:
                        d = jnp.dot(_unpack(h_p[13])[:, 0:64], _unpack(wd_p[FM // 2:F // 2, p * 128:(p + 1) * 128]),
                                    preferred_element_type=F32)
                    self.y = d if kt == 0 else self.y + d
                    if kt == 13:
                        g_v[pl.ds(self.r0, FB), p * 128:(p + 1) * 128] = _silu(self.y)

    class Tail:
        def __init__(self):
            self.n = 0

        def run_to(self, n_end):
            while self.n < min(n_end, 25 * NO):
                i, n, kt = self.n // 25, (self.n % 25) // 5, self.n % 5
                r0, r1, c0, c1 = i * TB, (i + 1) * TB, n * 128, (n + 1) * 128
                if self.n % 25 == 0:
                    self.o = ot_v[:, :, r0:r1].reshape(D, TB).astype(BF16).T
                d = jnp.dot(self.o[:, kt * 128:(kt + 1) * 128], wo_v[kt * 128:(kt + 1) * 128, c0:c1],
                            preferred_element_type=F32)
                self.s = d if kt == 0 else self.s + d
                if kt == 4:
                    out_v[r0:r1, c0:c1] = (x_v[r0:r1, c0:c1].astype(F32)
                                           + self.s * g_v[r0:r1, c0:c1]).astype(BF16)
                    for ci, o in enumerate(OUTS):
                        if o[1] == r1 and o[3] == c1:
                            out_copy(ci).start()
                self.n += 1

    def step(j, v, hook):
        e, t = v // NQT, v % NQT
        m8 = mr_v[v % NR]
        cq = jnp.broadcast_to(cq_v[j, e:e + 1, t * 128:(t + 1) * 128], (8, 128))
        acc = None
        for c in range(PP):
            r0, r1 = c * PL, (c + 1) * PL
            hook(v * PP + c)
            s = sr_v[v % NR, r0:r1, :].reshape(PL // 8, 8, 128)
            p = jnp.exp2((s - m8[None]) * cq[None]).reshape(PL, 128)
            d = lax.dot_general(ve_v[2 * j + e, :, r0:r1], p, NN, preferred_element_type=F32)
            acc = d if acc is None else acc + d
        if e == 0:
            o = acc * pl.reciprocal(acc[DH:DH + 1, :], approx=True)
            ot_v[j, 0:DH, t * 128:(t + 1) * 128] = o[0:DH, :]
        else:
            o = acc * pl.reciprocal(acc[0:1, :], approx=True)
            ot_v[j, DH:2 * DH, t * 128:(t + 1) * 128] = o[4:24, :]

    def body(j, last):
        qk, ffn, tail = QK(j, LU), FFN(j), Tail()
        cb1s, cb0s = CB(j, 1), CB(j + 1, 0)
        npos = NV * PP
        lead = LU / UQ + (QE - 1) * NV + 1
        a1 = (NQT - lead - CGAP) * PP
        b0, b1 = (NQT - LU / UQ + 0.5) * PP, (NV - lead - CGAP) * PP

        def hook(n):
            end = LU + min(NV * UQ, int(math.ceil((n + 1) * UQ / PP * QE - 1e-9)))
            if last:
                end = min(end, NV * UQ)
            assert (end - 1) // UQ - NR < n // PP
            assert (end - 1) // UQ < NQT or cb1s.n == CB.NPC
            assert (end - 1) // UQ < NV or cb0s.n == CB.NPC
            qk.run_to(end)
            ffn.run_to(FH + (NFT - FH) * (n + 1) / (npos * (LFE if last else 1.0)))
            cb1s.run_to(int(CB.NPC * (n + 1) / a1))
            if not last:
                if qk.n >= NQT * UQ:
                    cb0s.run_to(int(CB.NPC * (n + 1 - b0) / (b1 - b0)))
            else:
                ready = (max(0, n // PP - NQT) * 128 // TB) * 25
                want = (n / PP - NQT - TB // 128 - TLAG + 1) * 128 / TB * 25
                tail.run_to(min(ready, int(want)))

        for v in range(NV):
            step(j, v, hook)
        assert ffn.n == NFT and (last or qk.n == LU + NV * UQ)
        if last:
            tail.run_to(25 * NO)

    def att_body(j, carry):
        body(j, False)
        return carry

    CB(0, 0).run_to(CB.NPC)
    QK(0, 0).run_to(LU)
    lax.fori_loop(0, NP - 1, att_body, 0)
    body(NP - 1, True)

    for i in range(len(OUTS)):
        out_copy(i).wait()


@jax.jit
def pallas_recurrent_scan__mha_block__swiglu_ffn__prompt_kernel(
    A_x: jax.Array,
    A_wqkv: jax.Array,
    A_wo: jax.Array,
    B_x: jax.Array,
    B_w_gate: jax.Array,
    B_w_up: jax.Array,
    B_w_down: jax.Array,
):
    del B_x
    hbm_spec = pl.BlockSpec(memory_space=pltpu.MemorySpace.HBM)
    out = pl.pallas_call(
        _kernel,
        out_shape=jax.ShapeDtypeStruct((S, D), BF16),
        in_specs=[hbm_spec] * 6,
        out_specs=hbm_spec,
        scratch_shapes=[
            pltpu.VMEM((S, D), BF16),
            pltpu.VMEM((D, 3 * D), BF16),
            pltpu.VMEM((D, D), BF16),
            pltpu.VMEM((2 * F, D), BF16),
            pltpu.VMEM((F, D), BF16),
            pltpu.VMEM((S // 2, D), U32),
            pltpu.VMEM((D // 2, 2 * F), U32),
            pltpu.VMEM((F // 2, D), U32),
            pltpu.VMEM((D, D), U32),
            pltpu.VMEM((128, S), F32),
            pltpu.VMEM((H, S // 4, 128), U32),
            pltpu.VMEM((S, 128), F32),
            pltpu.VMEM((S, 128), F32),
            pltpu.VMEM((S, 128), F32),
            pltpu.VMEM((H, 32, S), U32),
            pltpu.VMEM((NP, 8, S), F32),
            pltpu.VMEM((H, 24, S), F32),
            pltpu.VMEM((NP, 2 * DH, S), F32),
            pltpu.VMEM((NR, S, 128), F32),
            pltpu.VMEM((NR, 8, 128), F32),
            pltpu.VMEM((14, FB // 2, 128), U32),
            pltpu.VMEM((S, D), F32),
            pltpu.VMEM((S, D), BF16),
            pltpu.SemaphoreType.DMA((SEM_O + len(OUTS),)),
        ],
        compiler_params=pltpu.CompilerParams(vmem_limit_bytes=100 * 1024 * 1024),
    )(A_x.reshape(S, D), A_wqkv, A_wo, B_w_gate.T, B_w_up.T, B_w_down)
    return out.reshape(1, S, D)
```

```python
import math

import jax
import jax.numpy as jnp
from jax import lax
import jax.experimental.pallas as pl
import jax.experimental.pallas.tpu as pltpu

S = 2048
D = 640
H = 32
DH = 20
F = 1728
FM = 1664
EPS = 1e-5
LOG2E = math.log2(math.e)

NN = (((1,), (0,)), ((), ()))
NT = (((1,), (1,)), ((), ()))
F32 = jnp.float32
BF16 = jnp.bfloat16
U32 = jnp.uint32
I32 = jnp.int32
I8 = jnp.int8

NP = H // 2
FB = S // NP
NQT = S // 128
NV = 2 * NQT
NR = 8
QL = 1024
PL = 128
UQ = S // QL
PP = S // PL
LU = 3 * UQ
QE = 1.04
FH = 2
NFT = 205
CBR = 16
CGAP = 4.0
LFE = 0.6
TLAG = 1.5
TB = 256
NO = S // TB
OUTS = [(0, 768, 0, D), (768, 1536, 0, D), (1536, 1792, 0, D), (1792, S, 0, 384), (1792, S, 384, D)]

RB = 256
QB = 128
MH = 16
XCH = [0, 1, 2, 4, 8]
B1, B2, B3, B4, NV0, B5 = 3, 8, 16, 26, 30, 14
LNS = 7
VKEEP = 5
VB5 = 2
NX = len(XCH) - 1
SEM_W = NX
SEM_O = NX + 8

BASE = 242.0
YMAX = 2770.0
MAGIC = 12582912.0


def _silu(x):
    return x * pl.reciprocal(1.0 + jnp.exp2(x * (-LOG2E)), approx=True)


def _pack(x):
    return pltpu.bitcast(x.astype(BF16), U32)


def _unpack(x):
    return pltpu.bitcast(x, BF16)


def _colmax8(s):
    return jnp.max(s.reshape(s.shape[0] // 8, 8, s.shape[1]), axis=0)


def _sumsq(w):
    w = w.astype(F32)
    return jnp.broadcast_to(jnp.sum(w * w, axis=0, keepdims=True), (8, w.shape[1]))


def _digits(v, e, is_q):
    n = v.shape[1]
    row = lax.broadcasted_iota(I32, (8, n), 0)
    if e == 0:
        v = jnp.concatenate([v[0:16], jnp.where(row < 4, v[16:24], 0.0)], axis=0)
    else:
        v = jnp.concatenate([jnp.where(row >= 4, v[0:8], 0.0), v[8:24]], axis=0)
    amax = jnp.maximum(jnp.max(jnp.abs(v), axis=0, keepdims=True), 1e-30)
    z = v * ((YMAX / BASE) * pl.reciprocal(amax, approx=True))
    hi = z + MAGIC
    a = hi - MAGIC
    f = z - a
    top = a * 11.0 + MAGIC
    lo = f * BASE + MAGIC
    lh = f * BASE ** 0.5 + MAGIC
    mid = [hi, lo] if is_q else [lo, hi]
    w = jnp.concatenate([top, top] + mid + [lh, jnp.zeros((8, n), F32)], axis=0)
    return amax, pltpu.bitcast(w, I32)


def _kernel(x_hbm, wqkv_hbm, wo_hbm, wg_hbm, wu_hbm, wd_hbm, out_hbm,
            x_v, wqkv_v, wo_v, wgu_v, wd_v,
            xn_p, wgu_p, wd_p, wt_p, sc_v, k_p, ck_v, cb0, cb1, q_p, cq_v, ve_v, ot_v,
            sr_v, mr_v, h_p, g_v, out_v, sems):
    def x_copy(i):
        r0, r1 = XCH[i] * RB, XCH[i + 1] * RB
        return pltpu.make_async_copy(x_hbm.at[r0:r1, :], x_v.at[r0:r1, :], sems.at[i])

    def out_copy(i):
        r0, r1, c0, c1 = OUTS[i]
        return pltpu.make_async_copy(out_v.at[r0:r1, c0:c1], out_hbm.at[r0:r1, c0:c1], sems.at[SEM_O + i])

    w_copies = [
        pltpu.make_async_copy(wqkv_hbm.at[:, 2 * D:3 * D], wqkv_v.at[:, 2 * D:3 * D], sems.at[SEM_W]),
        pltpu.make_async_copy(wqkv_hbm.at[:, D:2 * D], wqkv_v.at[:, D:2 * D], sems.at[SEM_W + 1]),
        pltpu.make_async_copy(wqkv_hbm.at[:, 0:D], wqkv_v.at[:, 0:D], sems.at[SEM_W + 2]),
        pltpu.make_async_copy(wg_hbm, wgu_v.at[0:F, :], sems.at[SEM_W + 3]),
        pltpu.make_async_copy(wu_hbm.at[FM:F, :], wgu_v.at[F:F + 64, :], sems.at[SEM_W + 4]),
        pltpu.make_async_copy(wu_hbm.at[0:FM, :], wgu_v.at[F + 64:2 * F, :], sems.at[SEM_W + 5]),
        pltpu.make_async_copy(wd_hbm, wd_v, sems.at[SEM_W + 6]),
        pltpu.make_async_copy(wo_hbm, wo_v, sems.at[SEM_W + 7]),
    ]

    def layernorm(i):
        r0 = i * RB
        x = x_v[r0:r0 + RB, :].astype(F32)
        mu = jnp.sum(x, axis=-1, keepdims=True) * (1.0 / D)
        xc = x - mu
        var = jnp.sum(xc * xc, axis=-1, keepdims=True) * (1.0 / D)
        xn_p[r0 // 2:(r0 + RB) // 2, :] = _pack(xc * lax.rsqrt(var + EPS))

    def balanced_transpose(t):
        wq = wqkv_v[:, t * 128:(t + 1) * 128]
        wk = wqkv_v[:, D + t * 128:D + (t + 1) * 128]
        nq = pltpu.bitcast(_sumsq(wq), I32)
        nk = pltpu.bitcast(_sumsq(wk), I32)
        ex = (nk - nq + (1 << 24)) >> 25
        ex = jnp.concatenate([ex] * 16, axis=0).T
        bq = pltpu.bitcast((127 + ex) << 23, F32)
        bk = pltpu.bitcast((127 - ex) << 23, F32)
        wt_p[t * 64:(t + 1) * 64, :] = _pack(wq.T.astype(F32) * jnp.concatenate([bq] * 5, axis=1))
        wt_p[(5 + t) * 64:(6 + t) * 64, :] = _pack(wk.T.astype(F32) * jnp.concatenate([bk] * 5, axis=1))

    def qk_piece(is_q, i, n):
        r0 = i * QB
        xn = _unpack(xn_p[r0 // 2:(r0 + QB) // 2, :])
        w0 = ((0 if is_q else D) + n * MH * DH) // 2
        yt = lax.dot_general(_unpack(wt_p[w0:w0 + MH * DH // 2, :]), xn, NT, preferred_element_type=F32)
        for hl in range(MH):
            h = n * MH + hl
            g0 = (hl * DH) // 8
            amax, w = _digits(yt[8 * g0:8 * g0 + 24], h % 2, is_q)
            if is_q:
                q_p[h, :, r0:r0 + QB] = pltpu.bitcast(w.astype(I8), U32)
                cq_v[h // 2, h % 2:h % 2 + 1, r0:r0 + QB] = amax * (BASE / YMAX ** 2 * DH ** -0.5 * LOG2E)
            else:
                k_p[h, r0 // 4:(r0 + QB) // 4, :] = pltpu.bitcast(w.astype(jnp.int16).T.astype(I8), U32)
                sc_v[h:h + 1, r0:r0 + QB] = amax
        if not is_q and (n + 1) * MH == H:
            ck_v[r0:r0 + QB, :] = sc_v[:, r0:r0 + QB].T

    def store_v(r0, n, y):
        yt = y.T
        row = lax.broadcasted_iota(I32, (8, RB), 0)
        for r in range(16):
            j, g = (16 * n + r) // 5, (16 * n + r) % 5
            v = yt[8 * r:8 * r + 8]
            if g < 2:
                ve_v[2 * j, 8 * g:8 * g + 8, r0:r0 + RB] = v
            elif g > 2:
                ve_v[2 * j + 1, 8 * g - 16:8 * g - 8, r0:r0 + RB] = v
            else:
                ve_v[2 * j, 16:24, r0:r0 + RB] = jnp.where(row < 4, v, 1.0)
                ve_v[2 * j + 1, 0:8, r0:r0 + RB] = jnp.where(row >= 4, v, 1.0)

    pend = []

    def v_piece(i, n):
        xn = _unpack(xn_p[i * RB // 2:(i + 1) * RB // 2, :])
        y = jnp.dot(xn, wqkv_v[:, 2 * D + n * 128:2 * D + (n + 1) * 128], preferred_element_type=F32)
        pend.append((i * RB, n, y))
        if len(pend) > 1:
            store_v(*pend.pop(0))

    x_copy(0).start()
    w_copies[0].start()
    x_copy(1).start()
    sc_v[H:128, :] = jnp.zeros((128 - H, S), F32)
    x_copy(0).wait()
    layernorm(0)
    w_copies[0].wait()
    x_copy(2).start()
    x_copy(3).start()
    for c in w_copies[1:]:
        c.start()

    vs = [(i, n) for i in range(S // RB) for n in range(5)]
    for cnt in range(NV0):
        if cnt == B1:
            x_copy(1).wait()
            layernorm(1)
        if cnt == B2:
            x_copy(2).wait()
            layernorm(2)
            layernorm(3)
        if cnt == B3:
            x_copy(3).wait()
            for i in range(4, LNS):
                layernorm(i)
        if cnt == B4:
            w_copies[1].wait()
            w_copies[2].wait()
            for i in range(LNS, S // RB):
                layernorm(i)
            for t in range(5):
                balanced_transpose(t)
        v_piece(*vs.pop(0))
    pieces = [(i, n) for i in range(S // QB) for n in range(H // MH)]
    npc, nv = len(pieces), len(vs)
    wjobs = [(0, t) for t in range(27)] + [(1, t) for t in range(14)]
    for cnt, (i, n) in enumerate(pieces):
        if cnt == B5:
            for _ in range(VB5):
                v_piece(*vs.pop(0))
            for c in w_copies[3:]:
                c.wait()
        qk_piece(True, i, n)
        qk_piece(False, i, n)
        while cnt >= B5 and len(wjobs) > 41 * (1.0 - (cnt + 1 - B5) / (npc - B5)):
            kind, t = wjobs.pop(0)
            if kind == 0:
                wgu_p[:, t * 128:(t + 1) * 128] = pltpu.bitcast(wgu_v[t * 128:(t + 1) * 128, :].T, U32)
            else:
                r1 = min(F, (t + 1) * 128)
                wd_p[t * 64:r1 // 2, :] = pltpu.bitcast(wd_v[t * 128:r1, :], U32)
        while nv - len(vs) - (VB5 if cnt >= B5 else 0) < (nv - VKEEP - VB5) * (cnt + 1) / npc:
            v_piece(*vs.pop(0))
    assert not wjobs
    while len(vs) > 1:
        v_piece(*vs.pop(0))

    cbuf = (cb0, cb1)

    class CB:
        NPC = S // CBR

        def __init__(self, j, e):
            self.j, self.e, self.n = j, e, 0

        def run_to(self, n_end):
            while self.n < min(n_end, self.NPC):
                r0, r1 = self.n * CBR, (self.n + 1) * CBR
                cbuf[self.e][r0:r1, :] = jnp.take_along_axis(
                    ck_v[r0:r1, :], jnp.full((CBR, 128), 2 * self.j + self.e, I32), axis=1)
                self.n += 1

    class QK:
        def __init__(self, j, n):
            self.j, self.n = j, n

        def run_to(self, n_end):
            while self.n < n_end:
                v, kq = self.n // UQ, self.n % UQ
                j, e, t = self.j + v // NV, (v % NV) // NQT, v % NQT
                r0, r1 = kq * QL, (kq + 1) * QL
                q = pltpu.bitcast(q_p[2 * j + e, :, t * 128:(t + 1) * 128], I8)
                k = pltpu.bitcast(k_p[2 * j + e, r0 // 4:r1 // 4, :], I8)
                s = lax.dot_general(k, q, NN, preferred_element_type=I32).astype(F32)
                s = s * cbuf[e][r0:r1, :]
                sr_v[v % NR, r0:r1, :] = s
                mc = _colmax8(s)
                self.mx = mc if kq == 0 else jnp.maximum(self.mx, mc)
                if r1 == S:
                    mr_v[v % NR] = jnp.broadcast_to(jnp.max(self.mx, axis=0, keepdims=True), (8, 128))
                self.n += 1

    class FFN:
        def __init__(self, j):
            self.n = 0
            self.r0 = j * FB if isinstance(j, int) else pl.multiple_of(j * FB, FB)
            self.p0 = j * (FB // 2) if isinstance(j, int) else pl.multiple_of(j * (FB // 2), FB // 2)
            cols = [("m", 13)]
            for p in range(13):
                cols += [("g", p), ("u", p)]
            self.tiles = [(kind, p, kt) for (kind, p) in cols for kt in range(5)]
            self.tiles += [("d", n, kt) for n in range(5) for kt in range(14)]

        def run_to(self, n_end):
            while self.n < min(n_end, NFT):
                kind, p, kt = self.tiles[self.n]
                self.n += 1
                if kind != "d":
                    xn = _unpack(xn_p[pl.ds(self.p0, FB // 2), kt * 128:(kt + 1) * 128])
                    t = p if kind != "u" else 14 + p
                    w = _unpack(wgu_p[kt * 64:(kt + 1) * 64, t * 128:(t + 1) * 128])
                    d = jnp.dot(xn, w, preferred_element_type=F32)
                    self.y = y = d if kt == 0 else self.y + d
                    if kt == 4:
                        if kind == "g":
                            self.gate = _silu(y)
                        elif kind == "u":
                            h_p[p] = _pack(self.gate * y)
                        else:
                            h_p[13] = _pack(_silu(y) * pltpu.roll(y, 64, 1))
                else:
                    if kt < 13:
                        d = jnp.dot(_unpack(h_p[kt]), _unpack(wd_p[kt * 64:(kt + 1) * 64, p * 128:(p + 1) * 128]),
                                    preferred_element_type=F32)
                    else:
                        d = jnp.dot(_unpack(h_p[13])[:, 0:64], _unpack(wd_p[FM // 2:F // 2, p * 128:(p + 1) * 128]),
                                    preferred_element_type=F32)
                    self.y = d if kt == 0 else self.y + d
                    if kt == 13:
                        g_v[pl.ds(self.r0, FB), p * 128:(p + 1) * 128] = _silu(self.y)

    class Tail:
        def __init__(self):
            self.n = 0

        def run_to(self, n_end):
            while self.n < min(n_end, 25 * NO):
                i, n, kt = self.n // 25, (self.n % 25) // 5, self.n % 5
                r0, r1, c0, c1 = i * TB, (i + 1) * TB, n * 128, (n + 1) * 128
                if self.n % 25 == 0:
                    self.o = ot_v[:, :, r0:r1].reshape(D, TB).astype(BF16).T
                d = jnp.dot(self.o[:, kt * 128:(kt + 1) * 128], wo_v[kt * 128:(kt + 1) * 128, c0:c1],
                            preferred_element_type=F32)
                self.s = d if kt == 0 else self.s + d
                if kt == 4:
                    out_v[r0:r1, c0:c1] = (x_v[r0:r1, c0:c1].astype(F32)
                                           + self.s * g_v[r0:r1, c0:c1]).astype(BF16)
                    for ci, o in enumerate(OUTS):
                        if o[1] == r1 and o[3] == c1:
                            out_copy(ci).start()
                self.n += 1

    def step(j, v, hook):
        e, t = v // NQT, v % NQT
        m8 = mr_v[v % NR]
        cq = jnp.broadcast_to(cq_v[j, e:e + 1, t * 128:(t + 1) * 128], (8, 128))
        acc = None
        for c in range(PP):
            r0, r1 = c * PL, (c + 1) * PL
            hook(v * PP + c)
            s = sr_v[v % NR, r0:r1, :].reshape(PL // 8, 8, 128)
            p = jnp.exp2((s - m8[None]) * cq[None]).reshape(PL, 128)
            d = lax.dot_general(ve_v[2 * j + e, :, r0:r1], p, NN, preferred_element_type=F32)
            acc = d if acc is None else acc + d
        if e == 0:
            o = acc * pl.reciprocal(acc[DH:DH + 1, :], approx=True)
            ot_v[j, 0:DH, t * 128:(t + 1) * 128] = o[0:DH, :]
        else:
            o = acc * pl.reciprocal(acc[0:1, :], approx=True)
            ot_v[j, DH:2 * DH, t * 128:(t + 1) * 128] = o[4:24, :]

    def body(j, last):
        qk, ffn, tail = QK(j, LU), FFN(j), Tail()
        cb1s, cb0s = CB(j, 1), CB(j + 1, 0)
        npos = NV * PP
        lead = LU / UQ + (QE - 1) * NV + 1
        a1 = (NQT - lead - CGAP) * PP
        b0, b1 = (NQT - LU / UQ + 0.5) * PP, (NV - lead - CGAP) * PP

        def hook(n):
            end = LU + min(NV * UQ, int(math.ceil((n + 1) * UQ / PP * QE - 1e-9)))
            if last:
                end = min(end, NV * UQ)
            assert (end - 1) // UQ - NR < n // PP
            assert (end - 1) // UQ < NQT or cb1s.n == CB.NPC
            assert (end - 1) // UQ < NV or cb0s.n == CB.NPC
            qk.run_to(end)
            ffn.run_to(FH + (NFT - FH) * (n + 1) / (npos * (LFE if last else 1.0)))
            cb1s.run_to(int(CB.NPC * (n + 1) / a1))
            if not last:
                if qk.n >= NQT * UQ:
                    cb0s.run_to(int(CB.NPC * (n + 1 - b0) / (b1 - b0)))
            else:
                ready = (max(0, n // PP - NQT) * 128 // TB) * 25
                want = (n / PP - NQT - TB // 128 - TLAG + 1) * 128 / TB * 25
                tail.run_to(min(ready, int(want)))

        for v in range(NV):
            step(j, v, hook)
        assert ffn.n == NFT and (last or qk.n == LU + NV * UQ)
        if last:
            tail.run_to(25 * NO)

    def att_body(j, carry):
        body(j, False)
        return carry

    CB(0, 0).run_to(CB.NPC)
    qk0 = QK(0, 0)
    qk0.run_to(2)
    v_piece(*vs.pop(0))
    qk0.run_to(LU)
    store_v(*pend.pop(0))
    assert not vs and not pend
    lax.fori_loop(0, NP - 1, att_body, 0)
    body(NP - 1, True)

    for i in range(len(OUTS)):
        out_copy(i).wait()


@jax.jit
def pallas_recurrent_scan__mha_block__swiglu_ffn__prompt_kernel(
    A_x: jax.Array,
    A_wqkv: jax.Array,
    A_wo: jax.Array,
    B_x: jax.Array,
    B_w_gate: jax.Array,
    B_w_up: jax.Array,
    B_w_down: jax.Array,
):
    del B_x
    hbm_spec = pl.BlockSpec(memory_space=pltpu.MemorySpace.HBM)
    out = pl.pallas_call(
        _kernel,
        out_shape=jax.ShapeDtypeStruct((S, D), BF16),
        in_specs=[hbm_spec] * 6,
        out_specs=hbm_spec,
        scratch_shapes=[
            pltpu.VMEM((S, D), BF16),
            pltpu.VMEM((D, 3 * D), BF16),
            pltpu.VMEM((D, D), BF16),
            pltpu.VMEM((2 * F, D), BF16),
            pltpu.VMEM((F, D), BF16),
            pltpu.VMEM((S // 2, D), U32),
            pltpu.VMEM((D // 2, 2 * F), U32),
            pltpu.VMEM((F // 2, D), U32),
            pltpu.VMEM((D, D), U32),
            pltpu.VMEM((128, S), F32),
            pltpu.VMEM((H, S // 4, 128), U32),
            pltpu.VMEM((S, 128), F32),
            pltpu.VMEM((S, 128), F32),
            pltpu.VMEM((S, 128), F32),
            pltpu.VMEM((H, 32, S), U32),
            pltpu.VMEM((NP, 8, S), F32),
            pltpu.VMEM((H, 24, S), F32),
            pltpu.VMEM((NP, 2 * DH, S), F32),
            pltpu.VMEM((NR, S, 128), F32),
            pltpu.VMEM((NR, 8, 128), F32),
            pltpu.VMEM((14, FB // 2, 128), U32),
            pltpu.VMEM((S, D), F32),
            pltpu.VMEM((S, D), BF16),
            pltpu.SemaphoreType.DMA((SEM_O + len(OUTS),)),
        ],
        compiler_params=pltpu.CompilerParams(vmem_limit_bytes=100 * 1024 * 1024),
    )(A_x.reshape(S, D), A_wqkv, A_wo, B_w_gate.T, B_w_up.T, B_w_down)
    return out.reshape(1, S, D)
```
